```python
import os as _os
_os.environ.setdefault("JAX_PLATFORMS", "cpu")
import jax
import jax.numpy as jnp

def _softmax(x, axis=-1):
    return jax.nn.softmax(x, axis=axis)
def _gelu(x):
    return jax.nn.gelu(x, approximate=True)
def _silu(x):
    return jax.nn.silu(x)
def _sigmoid(x):
    return jax.nn.sigmoid(x)
def _layernorm(x, axis=-1, eps=1e-5):
    m = jnp.mean(x, axis=axis, keepdims=True)
    v = jnp.var(x, axis=axis, keepdims=True)
    return (x - m) / jnp.sqrt(v + eps)
def _scatter_add(tgt, idx, src, axis=0):
    return tgt.at[idx].add(src)
def _segment_sum(src, seg, n):
    return jax.ops.segment_sum(src, seg, n)
class _Rng:
    def __init__(self, key):
        self._k = key
    def _next(self):
        self._k, sub = jax.random.split(self._k)
        return sub
    def normal(self, shape):
        return jax.random.normal(self._next(), shape, dtype=jnp.bfloat16)
    def randint(self, lo, hi, shape):
        return jax.random.randint(self._next(), shape, lo, hi, dtype=jnp.int32)
    def uniform(self, shape, lo=0.0, hi=1.0):
        return jax.random.uniform(self._next(), shape, jnp.bfloat16, lo, hi)
    def permutation(self, n):
        return jax.random.permutation(self._next(), n)


kernel_name = 'standalone__se_block__vision'

def setup_inputs():
    _rng = _Rng(jax.random.key(int.from_bytes(__import__("os").urandom(4), "little")))
    _w = (lambda a: (lambda t: t.astype(jnp.bfloat16) if jnp.issubdtype(t.dtype, jnp.floating) else t)(jnp.asarray(a)))
    H = W = 384
    C = 192; r = max(C // 16, 4)
    return {
        "x": _w((lambda *s: _rng.normal(s) * 0.8)(1, H, W, C)),
        "w_down": _w((lambda *s: _rng.normal(s) * 0.8)(C, r)),
        "w_up": _w((lambda *s: _rng.normal(s) * 0.8)(r, C)),
    }

def reference(x, w_down, w_up):
    s = x.mean(axis=(1, 2))
    s = _sigmoid(_silu(s @ w_down) @ w_up)
    return x * s[:, None, None, :]
```

```python
import jax
import jax.numpy as jnp
from jax import lax
import jax.experimental.pallas as pl
import jax.experimental.pallas.tpu as pltpu

LANES = 128


@jax.jit
def pallas_standalone__se_block__vision_kernel(
    x: jax.Array,
    w_down: jax.Array,
    w_up: jax.Array,
):
    n, h, w, c = x.shape
    r = w_down.shape[1]
    assert n == 1
    K, WIN, A, PR, G = 4, 4, 6, 16, 16
    hs = h // A
    rows_per_stream = hs * c
    n_chunks = h // K

    def kernel(x_hbm, wd_hbm, wu_hbm, o_hbm, buf, wd_v, wu_v, acc_ref, wd_col, wu_col, gate_ref,
               rd_sems, w_sems, wr_sem):
        xf = x_hbm.reshape(h, c, w)
        bf = buf.reshape(h, c, w)

        def read(i, slot):
            return pltpu.make_async_copy(xf.at[pl.ds(i * K, K)], bf.at[pl.ds(i * K, K)], rd_sems.at[slot])

        wcp = [pltpu.make_async_copy(wd_hbm, wd_v, w_sems.at[0]),
               pltpu.make_async_copy(wu_hbm, wu_v, w_sems.at[1])]
        read(0, 0).start()
        for cp in wcp:
            cp.start()
        for i in range(1, WIN):
            read(i, i).start()
        for cp in wcp:
            cp.wait()

        def to_col(m):
            m = m.astype(jnp.float32)
            m = jnp.concatenate([m, jnp.zeros((r, 2 * LANES - c), jnp.float32)], axis=1)
            m = jnp.concatenate([m, jnp.zeros((LANES - r, 2 * LANES), jnp.float32)], axis=0)
            return m.T[:c]

        wd_col[...] = to_col(wd_v[...])
        wu_col[...] = to_col(wu_v[...])
        acc_ref[...] = jnp.zeros((c, LANES), jnp.float32)

        def accumulate(i):
            for g in range(c // G):
                rows = pl.ds(g * G, G)
                a = acc_ref[rows, :]
                for k in range(K):
                    v = bf[i * K + k, rows, :].astype(jnp.float32)
                    a = a + ((v[:, 0:128] + v[:, 128:256]) + v[:, 256:384])
                acc_ref[rows, :] = a

        def rbody(i, carry):
            slot = lax.rem(i, WIN)
            read(i, slot).wait()
            read(i + WIN, slot).start()
            accumulate(i)
            return carry

        lax.fori_loop(0, n_chunks - WIN, rbody, 0)
        for i in range(n_chunks - WIN, n_chunks):
            read(i, i % WIN).wait()
            accumulate(i)

        rnd = lambda t: t.astype(jnp.bfloat16).astype(jnp.float32)
        mean = rnd(jnp.sum(acc_ref[...], axis=1, keepdims=True) * (1.0 / (h * w)))
        hid = rnd(jnp.sum(mean * wd_col[...], axis=0, keepdims=True))
        hid = rnd(hid * jax.nn.sigmoid(hid))
        z = rnd(jnp.sum(wu_col[...] * hid, axis=1, keepdims=True))
        gate = rnd(jax.nn.sigmoid(z))
        gate_ref[...] = jnp.broadcast_to(gate, (c, LANES))

        def wbody(hh, carry):
            for g in range(c // PR):
                r0 = pl.multiple_of(hh * c + g * PR, 8)
                gg = gate_ref[pl.ds(g * PR, PR), :]
                gg = jnp.concatenate([gg] * (w // LANES), axis=1)
                for a in range(A):
                    v = buf[a, pl.ds(r0, PR), :].astype(jnp.float32)
                    buf[a, pl.ds(r0, PR), :] = (v * gg).astype(buf.dtype)
                pltpu.make_async_copy(buf.at[:, pl.ds(r0, PR), :], o_hbm.at[:, pl.ds(r0, PR), :], wr_sem).start()
            return carry

        lax.fori_loop(0, hs, wbody, 0)
        pltpu.make_async_copy(buf, o_hbm, wr_sem).wait()

    xt = jnp.transpose(x, (0, 1, 3, 2)).reshape(A, rows_per_stream, w)
    out = pl.pallas_call(
        kernel,
        out_shape=jax.ShapeDtypeStruct((A, rows_per_stream, w), x.dtype),
        in_specs=[pl.BlockSpec(memory_space=pltpu.HBM)] * 3,
        out_specs=pl.BlockSpec(memory_space=pltpu.HBM),
        scratch_shapes=[
            pltpu.VMEM((A, rows_per_stream, w), x.dtype),
            pltpu.VMEM((r, c), w_down.dtype),
            pltpu.VMEM((r, c), w_up.dtype),
            pltpu.VMEM((c, LANES), jnp.float32),
            pltpu.VMEM((c, LANES), jnp.float32),
            pltpu.VMEM((c, LANES), jnp.float32),
            pltpu.VMEM((c, LANES), jnp.float32),
            pltpu.SemaphoreType.DMA((WIN,)),
            pltpu.SemaphoreType.DMA((2,)),
            pltpu.SemaphoreType.DMA(()),
        ],
        compiler_params=pltpu.CompilerParams(vmem_limit_bytes=100 * 1024 * 1024),
        name="se_block",
    )(xt, w_down.T, w_up)
    return jnp.transpose(out.reshape(n, h, c, w), (0, 1, 3, 2))
```

```python
import functools

import jax
import jax.numpy as jnp
from jax import lax
import jax.experimental.pallas as pl
import jax.experimental.pallas.tpu as pltpu

LANES = 128
TILE = 8
PAIR = 2 * TILE
BAND = 8

READ_STREAMS = 4
READ_SPLIT = 3
STAGES = 3
EXTRA_ROWS = 416
PAIRS_PER_TAIL = 2

WRITE_STREAMS = 6
RANGE_PIECES = 64
PIECE_ROWS = 64


def _tree_sum(terms):
    while len(terms) > 1:
        pairs = [terms[i] + terms[i + 1] for i in range(0, len(terms) - 1, 2)]
        terms = pairs + terms[2 * len(pairs):]
    return terms[0]


def _rows(start, size):
    if not isinstance(start, int):
        start = pl.multiple_of(start, PAIR)
    return pl.ds(start, size)


def _divmod(i, n):
    if isinstance(i, int):
        return divmod(i, n)
    return lax.div(i, n), lax.rem(i, n)


@jax.jit
def pallas_standalone__se_block__vision_kernel(
    x: jax.Array,
    w_down: jax.Array,
    w_up: jax.Array,
):
    batch, height, width, channels = x.shape
    hidden = w_down.shape[1]
    w_tiles = width // LANES
    slice_rows = channels * w_tiles
    pair_rows = PAIR * w_tiles
    pairs = channels // PAIR
    bands = height // BAND
    band_rows = BAND * slice_rows
    assert batch == 1 and height % BAND == 0 and width % LANES == 0
    assert channels % (PAIR * PAIRS_PER_TAIL) == 0

    rounds = (height - 2 * BAND - 1) // (READ_STREAMS * BAND + 1)
    head_bands = bands - 2 - rounds * READ_STREAMS
    read_rows = slice_rows // READ_SPLIT
    extra_band, extra_slice = divmod(rounds, BAND)
    head_start = extra_slice * slice_rows + EXTRA_ROWS
    head_spans = [(extra_band, head_start, band_rows - head_start)]
    head_spans += [(band, 0, band_rows) for band in range(extra_band + 1, head_bands)]
    chunks = [(height - 2 * size, size) for size in (BAND >> i for i in range(BAND.bit_length()))]
    last_slice = band_rows - slice_rows
    tail_starts = range(0, pairs, PAIRS_PER_TAIL)
    end_spans = [
        (first // BAND, first % BAND * slice_rows, size * slice_rows) for first, size in chunks
    ]
    end_spans += [
        (bands - 1, last_slice + p * pair_rows, PAIRS_PER_TAIL * pair_rows) for p in tail_starts
    ]
    assert STAGES - 1 <= rounds < head_bands * BAND
    assert read_rows * READ_SPLIT == slice_rows and read_rows % PAIR == 0
    assert 0 < EXTRA_ROWS < slice_rows and EXTRA_ROWS % PAIR == 0

    phases = slice_rows // PIECE_ROWS
    band_pieces = BAND * phases
    groups = bands * band_pieces // (WRITE_STREAMS * RANGE_PIECES)
    assert slice_rows % PIECE_ROWS == 0 and phases <= RANGE_PIECES
    assert groups * WRITE_STREAMS * RANGE_PIECES == bands * band_pieces

    def spread_over_lanes(w, table_ref):
        lane_pad = -channels % LANES
        if lane_pad:
            w = jnp.concatenate([w, jnp.zeros((hidden, lane_pad), w.dtype)], axis=1)
        for r in range(hidden):
            table_ref[r] = jnp.broadcast_to(w[r:r + 1], (LANES, w.shape[1])).T[:channels]

    def add_w_tiles(v):
        v = v.astype(jnp.float32).reshape(PAIR // TILE, w_tiles, TILE, LANES)
        return _tree_sum([v[:, t] for t in range(w_tiles)]).reshape(PAIR, LANES)

    def advance(position, count):
        band, piece, phase = position
        band += count // band_pieces
        piece += count % band_pieces
        phase += count % phases
        wrapped = piece >= band_pieces
        return (
            jnp.where(wrapped, band + 1, band),
            jnp.where(wrapped, piece - band_pieces, piece),
            jnp.where(phase >= phases, phase - phases, phase),
        )

    def body(x_hbm, wd_hbm, wu_hbm, out_hbm,
             buf, stage, wd_raw, wu_raw, wd_ref, wu_ref, acc_ref, gate_ref,
             head_sems, round_sems, end_sems, stage_in_sems, stage_out_sems,
             write_sem, fence_sem):
        def read(band, start, size, sem):
            rows = _rows(start, size)
            return pltpu.make_async_copy(x_hbm.at[band, rows], buf.at[band, rows], sem)

        def slice_at(ref, h, size):
            band, i = _divmod(h, BAND)
            return ref.at[band, _rows(i * slice_rows, size)]

        def stage_in(h, size=slice_rows):
            slot = _divmod(h, STAGES)[1]
            return pltpu.make_async_copy(
                slice_at(x_hbm, h, size), stage.at[slot, pl.ds(0, size)], stage_in_sems.at[slot]
            )

        def stage_out(h, size=slice_rows):
            slot = _divmod(h, STAGES)[1]
            return pltpu.make_async_copy(
                stage.at[slot, pl.ds(0, size)], slice_at(buf, h, size), stage_out_sems.at[slot]
            )

        def round_bands(i):
            return pl.ds(head_bands + i * READ_STREAMS, READ_STREAMS)

        def start_round(i):
            def start_pieces(j, carry):
                read(round_bands(i), j * read_rows, read_rows, round_sems.at[i]).start()
                return carry

            lax.fori_loop(0, BAND * READ_SPLIT, start_pieces, 0)

        def add_slice(h, carry):
            band, i = _divmod(h, BAND)
            for p in range(pairs):
                v = buf[band, _rows(i * slice_rows + p * pair_rows, pair_rows), :]
                acc_ref[pl.ds(p * PAIR, PAIR), :] += add_w_tiles(v)
            return carry

        weight_reads = [
            pltpu.make_async_copy(wd_hbm, wd_raw, head_sems.at[0]),
            pltpu.make_async_copy(wu_hbm, wu_raw, head_sems.at[1]),
        ]
        head_reads = [read(*span, head_sems.at[2 + i]) for i, span in enumerate(head_spans)]
        end_reads = [read(*span, end_sems.at[i]) for i, span in enumerate(end_spans)]
        for copy in weight_reads + head_reads:
            copy.start()
        for h in range(STAGES - 1):
            stage_in(h).start()
        start_round(0)
        acc_ref[...] = jnp.zeros_like(acc_ref)
        for copy in weight_reads:
            copy.wait()
        spread_over_lanes(wd_raw[...].astype(jnp.float32) * (1.0 / (height * width)), wd_ref)
        spread_over_lanes(wu_raw[...].astype(jnp.float32), wu_ref)
        for copy in head_reads:
            copy.wait()
        lax.fori_loop(rounds + 1, head_bands * BAND, add_slice, 0)

        def finish_round(i, carry):
            stage_in(i).wait()
            stage_out(i).start()

            @pl.when(i > 0)
            def _():
                stage_out(i - 1).wait()
                add_slice(i - 1, carry)

            @pl.when(i + STAGES - 1 < rounds)
            def _():
                stage_in(i + STAGES - 1).start()

            @pl.when(i + STAGES - 1 == rounds)
            def _():
                stage_in(rounds, EXTRA_ROWS).start()

            @pl.when(i + 1 < rounds)
            def _():
                start_round(i + 1)

            @pl.when(i + 1 == rounds)
            def _():
                for copy in end_reads:
                    copy.start()
                stage_in(rounds, EXTRA_ROWS).wait()
                stage_out(rounds, EXTRA_ROWS).start()

            read(round_bands(i), 0, band_rows, round_sems.at[i]).wait()
            first = (head_bands + i * READ_STREAMS) * BAND
            return lax.fori_loop(first, first + READ_STREAMS * BAND, add_slice, carry)

        lax.fori_loop(0, rounds, finish_round, 0)
        for copy, (first, size) in zip(end_reads, chunks):
            if size == 2:
                stage_out(rounds - 1).wait()
                add_slice(rounds - 1, 0)
            if size == 1:
                stage_out(rounds, EXTRA_ROWS).wait()
                add_slice(rounds, 0)
            copy.wait()
            lax.fori_loop(first, first + size, add_slice, 0)

        partial = [[] for _ in range(hidden)]
        for copy, first_pair in zip(end_reads[len(chunks):], tail_starts):
            copy.wait()
            for p in range(first_pair, first_pair + PAIRS_PER_TAIL):
                rows = pl.ds(p * PAIR, PAIR)
                v = buf[bands - 1, pl.ds(last_slice + p * pair_rows, pair_rows), :]
                total = acc_ref[rows, :] + add_w_tiles(v)
                for r in range(hidden):
                    term = total * wd_ref[r, rows, :]
                    partial[r] += [term[:TILE], term[TILE:]]
            partial = [[_tree_sum(terms)] for terms in partial]

        squeezed = jnp.concatenate(
            [jnp.sum(terms[0], axis=0, keepdims=True) for terms in partial], axis=0
        )
        squeezed = jnp.sum(squeezed, axis=1, keepdims=True)
        squeezed = squeezed * jax.nn.sigmoid(squeezed)

        @functools.cache
        def tile_gate(g):
            rows = pl.ds(g * TILE, TILE)
            terms = [squeezed[r:r + 1] * wu_ref[r, rows, :] for r in range(hidden)]
            return jax.nn.sigmoid(_tree_sum(terms))

        def write_piece(band, piece, gate):
            rows = _rows(piece * PIECE_ROWS, PIECE_ROWS)
            scaled = buf[band, rows, :].astype(jnp.float32) * gate
            buf[band, rows, :] = scaled.astype(buf.dtype)
            pltpu.make_async_copy(buf.at[band, rows], out_hbm.at[band, rows], write_sem).start()

        tiles_per_piece = PIECE_ROWS // TILE
        for phase in range(phases):
            tiles = range(phase * tiles_per_piece, (phase + 1) * tiles_per_piece)
            gate = jnp.concatenate([tile_gate(t // w_tiles) for t in tiles], axis=0)
            for s in range(WRITE_STREAMS):
                first = s * RANGE_PIECES
                write_piece(*divmod(first + (phase - first) % phases, band_pieces), gate)
            pl.semaphore_signal(fence_sem, 1)
            pl.semaphore_wait(fence_sem, 1)
            gate_ref[pl.ds(phase * PIECE_ROWS, PIECE_ROWS), :] = gate

        def write_step(_, position):
            for s in range(WRITE_STREAMS):
                band, piece, phase = advance(position, s * RANGE_PIECES)
                write_piece(band, piece, gate_ref[_rows(phase * PIECE_ROWS, PIECE_ROWS), :])
            return advance(position, 1)

        def write_group(g, position):
            first = jnp.where(g == 0, phases, 0)
            position = lax.fori_loop(first, RANGE_PIECES, write_step, position)
            return advance(position, (WRITE_STREAMS - 1) * RANGE_PIECES)

        zero = jnp.int32(0)
        lax.fori_loop(0, groups, write_group, advance((zero, zero, zero), phases))
        pltpu.make_async_copy(buf, out_hbm, write_sem).wait()

    def kernel(*refs):
        pl.run_scoped(
            lambda *sems: body(*refs, *sems),
            pltpu.SemaphoreType.DMA((2 + len(head_spans),)),
            pltpu.SemaphoreType.DMA((rounds,)),
            pltpu.SemaphoreType.DMA((len(end_spans),)),
            pltpu.SemaphoreType.DMA((STAGES,)),
            pltpu.SemaphoreType.DMA((STAGES,)),
            pltpu.SemaphoreType.DMA(()),
            pltpu.SemaphoreType.REGULAR,
        )

    tiled = x.reshape(height, w_tiles, LANES, channels // TILE, TILE)
    tiled = tiled.transpose(0, 3, 1, 4, 2).reshape(bands, band_rows, LANES)
    out = pl.pallas_call(
        kernel,
        out_shape=jax.ShapeDtypeStruct((bands, band_rows, LANES), x.dtype),
        in_specs=[pl.BlockSpec(memory_space=pltpu.HBM)] * 3,
        out_specs=pl.BlockSpec(memory_space=pltpu.HBM),
        scratch_shapes=[
            pltpu.VMEM((bands, band_rows, LANES), x.dtype),
            pltpu.SMEM((STAGES, slice_rows, LANES), x.dtype),
            pltpu.VMEM((hidden, channels), w_down.dtype),
            pltpu.VMEM((hidden, channels), w_up.dtype),
            pltpu.VMEM((hidden, channels, LANES), jnp.float32),
            pltpu.VMEM((hidden, channels, LANES), jnp.float32),
            pltpu.VMEM((channels, LANES), jnp.float32),
            pltpu.VMEM((slice_rows, LANES), jnp.float32),
        ],
        compiler_params=pltpu.CompilerParams(vmem_limit_bytes=72 * 1024 * 1024),
        name="se_block",
    )(tiled, w_down.T, w_up)
    out = out.reshape(height, channels // TILE, w_tiles, TILE, LANES)
    return out.transpose(0, 2, 4, 1, 3).reshape(x.shape)
```
